```python
import jax
import jax.numpy as jnp

def _softmax(x, axis=-1):
    return jax.nn.softmax(x, axis=axis)
def _gelu(x):
    return jax.nn.gelu(x, approximate=True)
def _silu(x):
    return jax.nn.silu(x)
def _sigmoid(x):
    return jax.nn.sigmoid(x)
def _layernorm(x, axis=-1, eps=1e-5):
    m = jnp.mean(x, axis=axis, keepdims=True)
    v = jnp.var(x, axis=axis, keepdims=True)
    return (x - m) / jnp.sqrt(v + eps)
def _scatter_add(tgt, idx, src, axis=0):
    return tgt.at[idx].add(src)
def _segment_sum(src, seg, n):
    return jax.ops.segment_sum(src, seg, n)
class _Rng:
    def __init__(self, key):
        self._k = key
    def _next(self):
        self._k, sub = jax.random.split(self._k)
        return sub
    def normal(self, shape):
        return jax.random.normal(self._next(), shape, dtype=jnp.bfloat16)
    def randint(self, lo, hi, shape):
        return jax.random.randint(self._next(), shape, lo, hi, dtype=jnp.int32)
    def uniform(self, shape, lo=0.0, hi=1.0):
        return jax.random.uniform(self._next(), shape, jnp.bfloat16, lo, hi)
    def permutation(self, n):
        return jax.random.permutation(self._next(), n)


kernel_name = 'sequential_preLN__spectral_gfnet__swiglu_ffn__prompt'

def _fwd_setup_inputs():
    _rng = _Rng(jax.random.key(int.from_bytes(__import__("os").urandom(4), "little")))
    _w = (lambda a: (lambda t: t.astype(jnp.bfloat16) if jnp.issubdtype(t.dtype, jnp.floating) else t)(jnp.asarray(a)))
    def _A_setup():
        B, S, D = 1, 2048, 576
        Df = D // 2 + 1
        return {
            "x": _w((lambda *s: _rng.normal(s) * 0.05)(B, S, D)),
            "w_r": _w((lambda *s: _rng.normal(s) * 0.05)(S, Df) * 0.02),
            "w_i": _w((lambda *s: _rng.normal(s) * 0.05)(S, Df) * 0.02),
        }
    _A_in = _A_setup()

    def _B_setup():
        B, S, D, F = 1, 2048, 576, 4608
        return {
            "x": _w((lambda *s: _rng.normal(s) * 0.05)(B, S, D)),
            "w_gate": _w((lambda *s: _rng.normal(s) * 0.05)(D, F)),
            "w_up": _w((lambda *s: _rng.normal(s) * 0.05)(D, F)),
            "w_down": _w((lambda *s: _rng.normal(s) * 0.05)(F, D)),
        }
    _B_in = _B_setup()

    return {
        "A_x": _A_in["x"],
        "A_w_r": _A_in["w_r"],
        "A_w_i": _A_in["w_i"],
        "B_x": _B_in["x"],
        "B_w_gate": _B_in["w_gate"],
        "B_w_up": _B_in["w_up"],
        "B_w_down": _B_in["w_down"],
    }

def _fwd_reference(A_x, A_w_r, A_w_i, B_x, B_w_gate, B_w_up, B_w_down):
    def _A_ref(x, w_r, w_i):
        B, S, D = x.shape
        X = (lambda x, axes=(-2,-1): jnp.fft.rfft2(x.astype(jnp.float32), axes=axes))(x, axes=(-2, -1))
        W = w_r + 1j * w_i
        X = X * W
        y = (lambda x, s, axes=(-2,-1): jnp.fft.irfft2(x, s=s, axes=axes).astype(jnp.bfloat16))(X, (S, D), axes=(-2, -1))
        return y

    def _B_ref(x, w_gate, w_up, w_down):
        g = _silu(x @ w_gate)
        u = x @ w_up
        return (g * u) @ w_down

    x = A_x
    h = x + _A_ref(_layernorm(x, axis=-1), A_w_r, A_w_i)
    h2 = h + _B_ref(_layernorm(h, axis=-1), B_w_gate, B_w_up, B_w_down)
    return h2


def setup_inputs():
    _inp = _fwd_setup_inputs()
    _gk = jax.random.fold_in(jax.random.key(int.from_bytes(__import__("os").urandom(4), "little")), 2**31 - 1)
    _shapes = [[1, 2048, 576]]
    _dtypes = ['bfloat16']
    _gks = jax.random.split(_gk, len(_shapes))
    _gs = [jax.random.normal(k, s, dtype=jnp.dtype(d)) * 0.05 for k, s, d in zip(_gks, _shapes, _dtypes)]
    _inp["grad_out"] = _gs[0]
    return _inp

def reference(A_x, A_w_r, A_w_i, B_w_gate, B_w_up, B_w_down, B_x, grad_out):
    _const = dict(B_x=B_x)
    def _f(*_d):
        return _fwd_reference(**{'A_x': _d[0], 'A_w_r': _d[1], 'A_w_i': _d[2], 'B_w_gate': _d[3], 'B_w_up': _d[4], 'B_w_down': _d[5], **_const})
    _out, _vjp = jax.vjp(_f, A_x, A_w_r, A_w_i, B_w_gate, B_w_up, B_w_down)
    _grads = _vjp(grad_out)
    _out0 = jnp.asarray(_out)
    return (_out0, *[jnp.asarray(_g) for _g in _grads])
```

```python
import math

import numpy as np
import jax
import jax.numpy as jnp
from jax import lax
import jax.experimental.pallas as pl
import jax.experimental.pallas.tpu as pltpu

S, D, F = 2048, 576, 4608
DF = D // 2 + 1
NT = S // 128
KR = 304
FT = 256
NJ = F // FT
ST = 512
EPS = 1e-5
bf16, f32, u32 = jnp.bfloat16, jnp.float32, jnp.uint32

_CLASSES = [q for g in (1, 2, 3, 4) for q in (g, g + 9, 9 - g, 18 - g)] + [0, 9]
_CLASS_ROW = {q: 16 * i for i, q in enumerate(_CLASSES)}


def _constants():
    k2 = np.full((KR,), -1)
    for q, r0 in _CLASS_ROW.items():
        k2[r0:r0 + 16] = q + 18 * np.arange(16)
    k2[288] = 288
    b = np.arange(64)
    fwd = np.zeros((5, 128, 128))
    inv = np.zeros((5, 128, 128))
    for g in (1, 2, 3, 4):
        k = k2[64 * (g - 1):64 * g]
        th = 2 * np.pi * ((k[:, None] * b[None, :]) % D) / D
        c, s = np.cos(th), np.sin(th)
        sg = np.where(k % 9 == g, 1.0, -1.0)[:, None]
        m = np.block([[c, sg * s], [-s, sg * c]])
        fwd[g] = m
        inv[g] = m.T * (2.0 / D)
    k = k2[256:304]
    ok = (k >= 0)[:, None]
    th = 2 * np.pi * ((k[:, None] * b[None, :]) % D) / D
    m = np.concatenate([np.cos(th) * ok, -np.sin(th) * (ok & (k[:, None] % 288 != 0))], 0)
    fwd[0, :96, :64] = m
    w = np.where(k % 288 == 0, 1.0, 2.0) / D
    inv[0, :64, :96] = m.T * np.concatenate([w, w])[None, :]
    fwd[3, :, 64:] *= math.sin(2 * math.pi / 3)
    inv[3, 64:, :] *= math.sin(2 * math.pi / 3)
    n = np.arange(128)
    ms = np.zeros((16, 256, 256))
    for r in range(16):
        th = 2 * np.pi * ((n[:, None] * (r + 16 * n[None, :])) % S) / S
        c, s = np.cos(th), np.sin(th)
        ms[r] = np.block([[c, -s], [s, c]])
    md = np.concatenate([fwd, inv], 0)
    return md.astype(jnp.bfloat16), ms.astype(jnp.bfloat16)


_MD, _MS = _constants()
_C9 = [math.cos(2 * math.pi * i / 9) for i in range(9)]
_S9 = [math.sin(2 * math.pi * i / 9) for i in range(9)]


def _nn(a, b):
    return jnp.dot(a, b, preferred_element_type=f32)


def _nt(a, b):
    return lax.dot_general(a, b, (((1,), (1,)), ((), ())), preferred_element_type=f32)


def _dft9(z):
    s = {j: z[j] + z[9 - j] for j in (1, 2, 3, 4)}
    t = {j: z[9 - j] - z[j] for j in (1, 2, 3, 4)}
    q = s[1] + s[2] + s[4]
    e = z[0] + s[3]
    c = z[0] - 0.5 * s[3]
    t3 = _S9[3] * t[3]
    out = {0: e + q, 5: e - 0.5 * q, 6: t[1] - t[2] + t[4]}
    for k in (1, 2, 4):
        out[2 * k - 1] = c + _C9[k] * s[1] + _C9[2 * k % 9] * s[2] + _C9[4 * k % 9] * s[4]
        im = _S9[k] * t[1] + _S9[2 * k % 9] * t[2] + _S9[4 * k % 9] * t[4]
        out[2 * k] = im - t3 if k == 2 else im + t3
    return [out[i] for i in range(9)]


def _idft9(v):
    v0, r1, i1, r2, i2, r3, i3, r4, i4 = v
    q = r1 + r2 + r4
    e = v0 + r3
    c = v0 - 0.5 * r3
    y = {0: e + q}
    p3 = e - 0.5 * q
    m3 = _S9[3] * (i1 - i2 + i4)
    y[3], y[6] = p3 - m3, p3 + m3
    for a in (1, 2, 4):
        p = c + _C9[a] * r1 + _C9[2 * a % 9] * r2 + _C9[4 * a % 9] * r4
        m = _S9[a] * i1 + _S9[2 * a % 9] * i2 + _S9[4 * a % 9] * i4
        m = m - i3 if a == 2 else m + i3
        y[a], y[9 - a] = p - m, p + m
    return [y[i] for i in range(9)]


def _dft4(x):
    (ar, ai), (br, bi), (cr, ci), (dr, di) = x
    pr, pi, mr, mi = ar + cr, ai + ci, ar - cr, ai - ci
    qr, qi, nr, ni = br + dr, bi + di, br - dr, bi - di
    return [(pr + qr, pi + qi), (mr + ni, mi - nr), (pr - qr, pi - qi), (mr - ni, mi + nr)]


def _tw16(x, e):
    re, im = x
    if e == 0:
        return x
    if e == 4:
        return im, -re
    h = math.sqrt(0.5)
    if e == 2:
        return (re + im) * h, (im - re) * h
    if e == 6:
        return (im - re) * h, (re + im) * (-h)
    c, s = math.cos(2 * math.pi * e / 16), math.sin(2 * math.pi * e / 16)
    return re * c + im * s, im * c - re * s


def _dft16(x):
    t = [_dft4([x[a0 + 4 * a1] for a1 in range(4)]) for a0 in range(4)]
    out = [None] * 16
    for k1 in range(4):
        y = _dft4([_tw16(t[a0][k1], a0 * k1) for a0 in range(4)])
        for k0 in range(4):
            out[k1 + 4 * k0] = y[k0]
    return out


def _kernel(x_h, wr_h, wi_h, wg_h, wu_h, wd_h, g_h, md_h, ms_h,
            out_h, dx_h, dwr_h, dwi_h, dwg_h, dwu_h, dwd_h,
            xT, gT, wr, wi, wg, wu, wd, md, ms,
            outb, dxb, dwr, dwi, dwb,
            n2T, n2, gn, acc_o, acc_n, U, V, Z, Xs, Wp, A, T, st1, st2,
            s_x, s_g, s_c, s_w, s_dw, s_o):
    CH = 512
    NC = S // CH

    def cols(i, n):
        return pl.ds(i * n if isinstance(i, int) else pl.multiple_of(i * n, n), n)

    x_cp = [pltpu.make_async_copy(x_h.at[:, cols(c, CH)], xT.at[:, cols(c, CH)], s_x.at[c])
            for c in range(NC)]
    g_cp = pltpu.make_async_copy(g_h, gT, s_g)
    c_cp = [pltpu.make_async_copy(a, b, s_c.at[i])
            for i, (a, b) in enumerate(((md_h, md), (wr_h, wr), (wi_h, wi), (ms_h, ms)))]

    def w_cp(j):
        return [pltpu.make_async_copy(a.at[:, cols(j, FT)], b.at[j], s_w.at[i, j])
                for i, (a, b) in enumerate(((wg_h, wg), (wu_h, wu), (wd_h, wd)))]

    def dw_cp(j):
        return [pltpu.make_async_copy(dwb.at[j % 2, i], o.at[:, cols(j, FT)], s_dw.at[i, j % 2])
                for i, o in enumerate((dwg_h, dwu_h, dwd_h))]

    x_cp[0].start()
    c_cp[0].start()
    for cp in x_cp[1:]:
        cp.start()
    for cp in c_cp[1:]:
        cp.start()
    g_cp.start()
    for j in range(NJ):
        for cp in w_cp(j):
            cp.start()

    def colsum(v):
        return jnp.sum(v, axis=0, keepdims=True)

    def ln_stats(v):
        mu = colsum(v) * (1.0 / D)
        xc = v - mu
        return mu, lax.rsqrt(colsum(xc * xc) * (1.0 / D) + EPS)

    def d_fwd(t, val):
        for b0 in range(0, 64, 16):
            u = _dft9([val[64 * a + b0:64 * a + b0 + 16] for a in range(9)])
            for i in range(9):
                U[pl.ds((i + 8) % 9 * 64 + b0, 16), :] = u[i].astype(bf16)
        for g in (1, 2, 3, 4):
            z = _nn(md[g], U[pl.ds(128 * (g - 1), 128), :])
            Z[0, t, pl.ds(64 * (g - 1), 64), :] = z[:64]
            Z[1, t, pl.ds(64 * (g - 1), 64), :] = z[64:]
        z = _nn(md[0, :96, :64], U[pl.ds(512, 64), :])
        Z[0, t, pl.ds(256, 48), :] = z[:48]
        Z[1, t, pl.ds(256, 48), :] = z[48:]

    def d_inv(t):
        for g in (1, 2, 3, 4):
            r = pl.ds(64 * (g - 1), 64)
            y = jnp.concatenate([Z[0, t, r, :].astype(bf16), Z[1, t, r, :].astype(bf16)], axis=0)
            V[pl.ds(64 + 128 * (g - 1), 128), :] = _nn(md[5 + g], y)
        r = pl.ds(256, 48)
        y = jnp.concatenate([Z[0, t, r, :].astype(bf16), Z[1, t, r, :].astype(bf16)], axis=0)
        V[pl.ds(0, 64), :] = _nn(md[5, :64, :96], y)
        y = _idft9([V[pl.ds(64 * i, 64), :] for i in range(9)])
        return jnp.concatenate(y, axis=0)

    def s_radix16(inverse):
        p, q = (1, 0) if inverse else (0, 1)

        def body(i, _):
            r = pl.ds(pl.multiple_of(i * 8, 8), 8)
            y = _dft16([(Z[p, a, r, :], Z[q, a, r, :]) for a in range(16)])
            for a in range(16):
                Z[p, a, r, :] = y[a][0]
                Z[q, a, r, :] = y[a][1]
        lax.fori_loop(0, 37, body, None)

    def s_fwd(r):
        z = jnp.concatenate([Z[0, r].astype(bf16), Z[1, r].astype(bf16)], axis=1)
        return _nn(z, ms[r])

    def s_inv(r, yr, yi):
        y = _nt(jnp.concatenate([yr.astype(bf16), yi.astype(bf16)], axis=1), ms[r])
        Z[0, r] = y[:, :128]
        Z[1, r] = y[:, 128:]

    c_cp[0].wait()
    for c in range(NC):
        x_cp[c].wait()

        def a_body(i, _, c=c):
            t = c * (CH // 128) + i
            v = xT[:, cols(t, 128)].astype(f32)
            mu, rs = ln_stats(v)
            st1[0:1, cols(t, 128)] = mu
            st1[1:2, cols(t, 128)] = rs
            d_fwd(t, (v - mu) * rs)
        lax.fori_loop(0, CH // 128, a_body, None)
    s_radix16(False)

    c_cp[1].wait()
    c_cp[2].wait()

    def w1_body(t, _):
        c = cols(t, 128)
        A[0:144, :] = pltpu.bitcast(wr[0:288, c], u32)
        A[144:288, :] = pltpu.bitcast(wi[0:288, c], u32)
        rows = [A[pl.ds(144 * p + cc, 16, stride=9), :] for p in range(2) for cc in range(9)]
        nr = pltpu.bitcast(wr[288:289, c].astype(f32), u32)
        ni = pltpu.bitcast(wi[288:289, c].astype(f32), u32)
        m = jnp.concatenate(rows + [jnp.broadcast_to((nr >> 16) | ni, (8, 128)),
                                    jnp.zeros((88, 128), u32)], axis=0)
        for q in range(3):
            T[q, c, :] = m[128 * q:128 * q + 128].T
    lax.fori_loop(0, NT, w1_body, None)

    def lo(v):
        return pltpu.bitcast(v << 16, f32)

    def hi(v):
        return pltpu.bitcast(v & jnp.uint32(0xFFFF0000), f32)

    row16 = lax.broadcasted_iota(jnp.int32, (16, 128), 0)
    c_cp[3].wait()

    def c_body(r, _):
        m = jnp.concatenate([T[q, pl.ds(r, 128, stride=16), :].T for q in range(3)], axis=0)
        for p in range(2):
            for cc in range(9):
                v = m[144 * p + 16 * cc:144 * p + 16 * cc + 16]
                Wp[r, p, pl.ds(_CLASS_ROW[2 * cc], 16), :] = lo(v)
                Wp[r, p, pl.ds(_CLASS_ROW[2 * cc + 1], 16), :] = hi(v)
        ny = jnp.where(row16 == 0, m[288:304], jnp.uint32(0))
        Wp[r, 0, pl.ds(288, 16), :] = lo(ny)
        Wp[r, 1, pl.ds(288, 16), :] = hi(ny)
        x = s_fwd(r)
        Xs[r] = x.astype(bf16)
        xr, xi, w_r, w_i = x[:, :128], x[:, 128:], Wp[r, 0], Wp[r, 1]
        s_inv(r, xr * w_r - xi * w_i, xr * w_i + xi * w_r)
    lax.fori_loop(0, 16, c_body, None)
    s_radix16(True)
    g_cp.wait()

    def e_body(t, _):
        c = cols(t, 128)
        h = xT[:, c].astype(f32) + d_inv(t) * (1.0 / S)
        acc_o[:, c] = h
        acc_n[:, c] = jnp.zeros((D, 128), f32)
        mu, rs = ln_stats(h)
        st2[0:1, c] = rs
        n = (h - mu) * rs
        n2T[:, c] = n.astype(bf16)
        n2[c, :] = n.T.astype(bf16)
        gn[c, :] = gT[:, c].astype(f32).T.astype(bf16)
    lax.fori_loop(0, NT, e_body, None)

    def f_body(j, _):
        for cp in w_cp(j):
            cp.wait()

        @pl.when(j >= 2)
        def _():
            for cp in dw_cp(j - 2):
                cp.wait()

        def s1(i):
            r = cols(i, ST)
            a, u, dp = _nn(n2[r, :], wg[j]), _nn(n2[r, :], wu[j]), _nn(gn[r, :], wd[j])
            sig = 0.5 * jnp.tanh(0.5 * a) + 0.5
            sl = a * sig
            return ((sl * u).astype(bf16), (dp * u * (sig + sl * (1.0 - sig))).astype(bf16),
                    (dp * sl).astype(bf16))

        tot = None
        for i in range(S // ST):
            p, da, du = s1(i)
            r = cols(i, ST)
            acc_o[:, r] += _nt(wd[j], p)
            acc_n[:, r] += _nt(wg[j], da) + _nt(wu[j], du)
            new = [_nn(n2T[:, r], da), _nn(n2T[:, r], du), _nn(gT[:, r], p)]
            tot = new if tot is None else [a + b for a, b in zip(tot, new)]
        for i in range(3):
            dwb[j % 2, i] = tot[i].astype(bf16)
        for cp in dw_cp(j):
            cp.start()
    lax.fori_loop(0, NJ, f_body, None)

    def ln_bwd(dn, n, rs):
        return rs * (dn - colsum(dn) * (1.0 / D) - n * (colsum(dn * n) * (1.0 / D)))

    def a2_body(t, _):
        c = cols(t, 128)
        outb[:, c] = acc_o[:, c].astype(bf16)
        dh = gT[:, c].astype(f32) + ln_bwd(acc_n[:, c], n2T[:, c].astype(f32), st2[0:1, c])
        acc_n[:, c] = dh
        d_fwd(t, dh)
    lax.fori_loop(0, NT, a2_body, None)
    o_cp = pltpu.make_async_copy(outb, out_h, s_o.at[0])
    o_cp.start()
    s_radix16(False)

    rowk = lax.broadcasted_iota(jnp.int32, (KR, 128), 0)

    def bits(v):
        return pltpu.bitcast(v.astype(bf16).astype(f32), u32)

    def c2_body(r, _):
        gs = s_fwd(r)
        gr, gi, w_r, w_i = gs[:, :128], gs[:, 128:], Wp[r, 0], Wp[r, 1]
        s_inv(r, gr * w_r + gi * w_i, gi * w_r - gr * w_i)
        xr, xi = Xs[r, :, :128].astype(f32), Xs[r, :, 128:].astype(f32)
        sc = jnp.where((rowk == 256) | (rowk == 288), 1.0 / (S * D), 2.0 / (S * D))
        d = [bits((xr * gr + xi * gi) * sc), bits((xr * gi - xi * gr) * sc)]
        rows = []
        for p in range(2):
            for cc in range(9):
                a, b = _CLASS_ROW[2 * cc], _CLASS_ROW[2 * cc + 1]
                rows.append((d[p][a:a + 16] >> 16) | d[p][b:b + 16])
        rows += [(d[0][288:304] >> 16) | d[1][288:304], jnp.zeros((80, 128), u32)]
        m = jnp.concatenate(rows, axis=0)
        for q in range(3):
            T[q, pl.ds(r, 128, stride=16), :] = m[128 * q:128 * q + 128].T
    lax.fori_loop(0, 16, c2_body, None)

    def w2_body(t, _):
        c = cols(t, 128)
        m = jnp.concatenate([T[q, c, :].T for q in range(3)], axis=0)
        for p in range(2):
            for cc in range(9):
                A[pl.ds(144 * p + cc, 16, stride=9), :] = m[144 * p + 16 * cc:144 * p + 16 * cc + 16]
        dwr[0:288, c] = pltpu.bitcast(A[0:144, :], bf16)
        dwi[0:288, c] = pltpu.bitcast(A[144:288, :], bf16)
        dwr[288:289, c] = lo(m[288:289]).astype(bf16)
        dwi[288:289, c] = hi(m[288:289]).astype(bf16)
    lax.fori_loop(0, NT, w2_body, None)
    dwr_cp = pltpu.make_async_copy(dwr, dwr_h, s_o.at[1])
    dwi_cp = pltpu.make_async_copy(dwi, dwi_h, s_o.at[2])
    dwr_cp.start()
    dwi_cp.start()
    s_radix16(True)

    dx_cp = [pltpu.make_async_copy(dxb.at[:, cols(c, CH)], dx_h.at[:, cols(c, CH)], s_o.at[3 + c])
             for c in range(NC)]
    for c in range(NC):
        def e2_body(i, _, c=c):
            t = c * (CH // 128) + i
            k = cols(t, 128)
            rs = st1[1:2, k]
            n = (xT[:, k].astype(f32) - st1[0:1, k]) * rs
            dxb[:, k] = (acc_n[:, k] + ln_bwd(d_inv(t) * (1.0 / S), n, rs)).astype(bf16)
        lax.fori_loop(0, CH // 128, e2_body, None)
        dx_cp[c].start()

    for j in (NJ - 2, NJ - 1):
        for cp in dw_cp(j):
            cp.wait()
    for cp in [o_cp, dwr_cp, dwi_cp] + dx_cp:
        cp.wait()


@jax.jit
def pallas_sequential_preLN__spectral_gfnet__swiglu_ffn__prompt_kernel(
    A_x: jax.Array,
    A_w_r: jax.Array,
    A_w_i: jax.Array,
    B_x: jax.Array,
    B_w_gate: jax.Array,
    B_w_up: jax.Array,
    B_w_down: jax.Array,
    grad_out: jax.Array,
):
    del B_x
    sds = jax.ShapeDtypeStruct
    vm = pltpu.VMEM
    hbm = pl.BlockSpec(memory_space=pl.ANY)
    dma = pltpu.SemaphoreType.DMA
    out, dx, dwr, dwi, dwg, dwu, dwd = pl.pallas_call(
        _kernel,
        in_specs=[hbm] * 9,
        out_specs=[hbm] * 7,
        out_shape=[sds((D, S), bf16)] * 2 + [sds((DF, S), bf16)] * 2 + [sds((D, F), bf16)] * 3,
        scratch_shapes=[
            vm((D, S), bf16), vm((D, S), bf16), vm((DF, S), bf16), vm((DF, S), bf16),
            vm((NJ, D, FT), bf16), vm((NJ, D, FT), bf16), vm((NJ, D, FT), bf16),
            vm((10, 128, 128), bf16), vm((16, 256, 256), bf16),
            vm((D, S), bf16), vm((D, S), bf16), vm((DF, S), bf16), vm((DF, S), bf16),
            vm((2, 3, D, FT), bf16),
            vm((D, S), bf16), vm((S, D), bf16), vm((S, D), bf16),
            vm((D, S), f32), vm((D, S), f32),
            vm((D, 128), bf16), vm((D, 128), f32),
            vm((2, NT, KR, 128), f32), vm((16, KR, 256), bf16), vm((16, 2, KR, 128), f32),
            vm((288, 128), u32), vm((3, S, 128), u32), vm((8, S), f32), vm((8, S), f32),
            dma((4,)), dma, dma((4,)), dma((3, NJ)), dma((3, 2)), dma((7,)),
        ],
        compiler_params=pltpu.CompilerParams(vmem_limit_bytes=120 * 2**20),
    )(A_x[0].T, A_w_r.T, A_w_i.T, B_w_gate, B_w_up, B_w_down.T, grad_out[0].T, _MD, _MS)
    return out.T[None], dx.T[None], dwr.T, dwi.T, dwg, dwu, dwd.T
```

```python
import math

import numpy as np
import jax
import jax.numpy as jnp
from jax import lax
import jax.experimental.pallas as pl
import jax.experimental.pallas.tpu as pltpu

S, D, F = 2048, 576, 4608
DF = D // 2 + 1
NT = S // 128
KR = 304
FT = 256
NJ = F // FT
HS = 512
HF, HD = FT // 2, D // 2
NU = S // (2 * HS)
EPS = 1e-5
SPREAD = 3.0
bf16, f32, u32 = jnp.bfloat16, jnp.float32, jnp.uint32

_CLASSES = [q for g in (1, 2, 3, 4) for q in (g, g + 9, 9 - g, 18 - g)] + [0, 9]
_CLASS_ROW = {q: 16 * i for i, q in enumerate(_CLASSES)}


def _constants():
    k2 = np.full((KR,), -1)
    for q, r0 in _CLASS_ROW.items():
        k2[r0:r0 + 16] = q + 18 * np.arange(16)
    k2[288] = 288
    b = np.arange(64)
    fwd = np.zeros((5, 128, 128))
    inv = np.zeros((5, 128, 128))
    for g in (1, 2, 3, 4):
        k = k2[64 * (g - 1):64 * g]
        th = 2 * np.pi * ((k[:, None] * b[None, :]) % D) / D
        c, s = np.cos(th), np.sin(th)
        sg = np.where(k % 9 == g, 1.0, -1.0)[:, None]
        m = np.block([[c, sg * s], [-s, sg * c]])
        fwd[g] = m
        inv[g] = m.T * (2.0 / D)
    k = k2[256:304]
    ok = (k >= 0)[:, None]
    th = 2 * np.pi * ((k[:, None] * b[None, :]) % D) / D
    m = np.concatenate([np.cos(th) * ok, -np.sin(th) * (ok & (k[:, None] % 288 != 0))], 0)
    fwd[0, :96, :64] = m
    w = np.where(k % 288 == 0, 1.0, 2.0) / D
    inv[0, :64, :96] = m.T * np.concatenate([w, w])[None, :]
    fwd[3, :, 64:] *= math.sin(2 * math.pi / 3)
    inv[3, 64:, :] *= math.sin(2 * math.pi / 3)
    n = np.arange(128)
    ms = np.zeros((16, 256, 256))
    for r in range(16):
        ka = (n - r) % 16
        k1 = 128 * ka + (n - ka) % 128
        th = 2 * np.pi * ((n[:, None] * k1[None, :]) % S) / S
        c, s = np.cos(th), np.sin(th)
        ms[r] = np.block([[c, -s], [s, c]])
    md = np.concatenate([fwd, inv / S], 0)
    return md.astype(jnp.bfloat16), ms.astype(jnp.bfloat16)


_MD, _MS = _constants()
_C9 = [math.cos(2 * math.pi * i / 9) for i in range(9)]
_S9 = [math.sin(2 * math.pi * i / 9) for i in range(9)]


def _total(xs):
    xs = list(xs)
    for x in xs[1:]:
        xs[0] = xs[0] + x
    return xs[0]


def _nn(a, b):
    return jnp.dot(a, b, preferred_element_type=f32)


def _nt(a, b):
    return lax.dot_general(a, b, (((1,), (1,)), ((), ())), preferred_element_type=f32)


_SCALES = ((1.0, 2.0, 1.0), (2.0, 1.0, 1.0), (1.0, 1.0, 1.0), (2.0, 0.5, 0.5))
_PASSES = (((0, 5), "p2"), ((1, 5), (2, 5)), ((3, 5), "ph"), ((0, 1), (1, 1)),
           ((0, 2), "q2"), ((1, 2), (2, 2)), ((3, 2), "qh"), ((2, 1), (3, 1)),
           ((0, 3), (2, 3)), ((1, 3), (3, 3)), ((0, 6), (1, 6)), ((2, 6), (3, 6)),
           ((0, 4), (2, 4)), ((1, 4), (3, 4)), ((0, 7), (1, 7)), ((2, 7), (3, 7)))


def _lin(ca, a, cb, b):
    a = a if ca == 1 else ca * a
    return a + b if cb == 1 else a - b if cb == -1 else a + cb * b


def _left(slot, blk):
    if isinstance(slot, str):
        return blk(int(slot[0] == "q"), 512)
    n, m = slot
    u, _, g = _SCALES[n]
    x, y = 128 * n, 128 * n + 64
    if m == 3:
        return blk(0, x)
    if m == 4:
        return blk(1, y)
    a, c, b = {1: ((0, x), 1 / (u * g), (1, y)), 2: ((1, x), 1 / g, (1, y)),
               5: ((0, x), 1 / g, (0, y)), 6: ((1, x), -u, (0, x)),
               7: ((0, y), -1 / u, (1, y))}[m]
    return _lin(1, blk(*a), c, blk(*b))


def _right(slot, blk):
    if isinstance(slot, str):
        return _lin(-1 / 3, blk(0, 512), -2 / 3, blk(1, 512)) if slot[1] == "2" else \
            _lin(4 / 3, blk(0, 512), 2 / 3, blk(1, 512))
    n, m = slot
    u, v, g = _SCALES[n]
    x, y = 128 * n, 128 * n + 64
    if m == 2:
        return blk(0, x)
    if m == 5:
        return (-g / v) * blk(1, y)
    ca, a, cb, b = {1: (1, (0, x), g / v, (1, y)), 3: (1, (1, x), -g, (1, y)),
                    4: (1 / u, (0, y), -1 / (u * g), (0, x)), 6: (1, (1, x), v, (0, x)),
                    7: (1, (0, y), 1 / v, (1, y))}[m]
    return _lin(ca, blk(*a), cb, blk(*b))


_ORDER = (0, 1, 2, 3, 8, 9, 4, 5, 6, 12, 13, 7, 14, 15, 10, 11)


def _quadrants(p2, p1, ph, ia, q2, q1, qh, ib, g1, g2, s2, s3, f1, f2, s0, s1):
    c12 = (g1 + g2) - ((2.0 * p2 + p1) + 0.5 * ph)
    c21 = (q2 + q1) + ((qh + f1) + 2.0 * f2)
    c11 = ((p2 + p1) + (ph + ia)) + ((f1 + f2) + ib) + (s0 + s1)
    c22 = (2.0 * ((ia - q2) + g2) + (g1 - q1)) + (ib - 0.5 * qh) + (s2 + s3)
    return c11, c12, c21, c22


def _tn(a, b):
    return lax.dot_general(a, b, (((0,), (0,)), ((), ())), preferred_element_type=f32)


def _swiglu(a, b, dp):
    sig = 0.5 * jnp.tanh(0.5 * a) + 0.5
    sl = a * sig
    return dp * (b * (sig + sl * (1.0 - sig))), dp * sl, sl * b


def _balanced(sq):
    top, low = jnp.max(sq, keepdims=True), jnp.min(sq, keepdims=True)
    return jnp.where((top <= SPREAD * low) & (top > 1e-30) & (top < 1e30), 1.0, 0.0)


def _dft9(z):
    s = {j: z[j] + z[9 - j] for j in (1, 2, 3, 4)}
    t = {j: z[9 - j] - z[j] for j in (1, 2, 3, 4)}
    q = s[1] + s[2] + s[4]
    e = z[0] + s[3]
    c = z[0] - 0.5 * s[3]
    t3 = _S9[3] * t[3]
    out = {0: e + q, 5: e - 0.5 * q, 6: t[1] - t[2] + t[4]}
    for k in (1, 2, 4):
        out[2 * k - 1] = c + _C9[k] * s[1] + _C9[2 * k % 9] * s[2] + _C9[4 * k % 9] * s[4]
        im = _S9[k] * t[1] + _S9[2 * k % 9] * t[2] + _S9[4 * k % 9] * t[4]
        out[2 * k] = im - t3 if k == 2 else im + t3
    return [out[i] for i in range(9)]


def _idft9(v):
    v0, r1, i1, r2, i2, r3, i3, r4, i4 = v
    q = r1 + r2 + r4
    e = v0 + r3
    c = v0 - 0.5 * r3
    y = {0: e + q}
    p3 = e - 0.5 * q
    m3 = _S9[3] * (i1 - i2 + i4)
    y[3], y[6] = p3 - m3, p3 + m3
    for a in (1, 2, 4):
        p = c + _C9[a] * r1 + _C9[2 * a % 9] * r2 + _C9[4 * a % 9] * r4
        m = _S9[a] * i1 + _S9[2 * a % 9] * i2 + _S9[4 * a % 9] * i4
        m = m - i3 if a == 2 else m + i3
        y[a], y[9 - a] = p - m, p + m
    return [y[i] for i in range(9)]


def _dft4(x):
    (ar, ai), (br, bi), (cr, ci), (dr, di) = x
    pr, pi, mr, mi = ar + cr, ai + ci, ar - cr, ai - ci
    qr, qi, nr, ni = br + dr, bi + di, br - dr, bi - di
    return [(pr + qr, pi + qi), (mr + ni, mi - nr), (pr - qr, pi - qi), (mr - ni, mi + nr)]


def _tw16(x, e):
    re, im = x
    if e == 0:
        return x
    if e == 4:
        return im, -re
    h = math.sqrt(0.5)
    if e == 2:
        return (re + im) * h, (im - re) * h
    if e == 6:
        return (im - re) * h, (re + im) * (-h)
    c, s = math.cos(2 * math.pi * e / 16), math.sin(2 * math.pi * e / 16)
    return re * c + im * s, im * c - re * s


def _dft16(x):
    t = [_dft4([x[a0 + 4 * a1] for a1 in range(4)]) for a0 in range(4)]
    out = [None] * 16
    for k1 in range(4):
        y = _dft4([_tw16(t[a0][k1], a0 * k1) for a0 in range(4)])
        for k0 in range(4):
            out[k1 + 4 * k0] = y[k0]
    return out


def _kernel(x_h, wr_h, wi_h, wg_h, wu_h, wd_h, g_h, md_h, ms_h,
            out_h, dx_h, dwr_h, dwi_h, dwg_h, dwu_h, dwd_h,
            xT, gT, wr, wi, wg, wu, wd, md, ms,
            outb, dxb, dwr, dwi, dwb,
            n2T, n2Tc, gTc, n2c, gc, acc_o, acc_n, acc_w, Z, Xs, Wp, T, st1, st2,
            s_x, s_g, s_c, s_w, s_dw, s_o):
    CH = 512
    NC = S // CH

    def cols(i, n):
        return pl.ds(i * n if isinstance(i, int) else pl.multiple_of(i * n, n), n)

    def x_cp(c):
        return pltpu.make_async_copy(x_h.at[:, cols(c, CH)], xT.at[:, cols(c, CH)], s_x.at[c])

    g_cp = [pltpu.make_async_copy(g_h.at[:, cols(u, 2 * HS)], gT.at[:, cols(u, 2 * HS)], s_g.at[u])
            for u in range(NU)]
    c_cp = [pltpu.make_async_copy(a, b, s_c.at[i])
            for i, (a, b) in enumerate(((md_h, md), (wr_h, wr), (wi_h, wi),
                                        (ms_h.at[:8], ms.at[:8]), (ms_h.at[8:], ms.at[8:])))]

    def w_cp(j):
        return [pltpu.make_async_copy(a.at[:, cols(j, FT)], b.at[j], s_w.at[i, j])
                for i, (a, b) in enumerate(((wg_h, wg), (wu_h, wu), (wd_h, wd)))]

    def dw_cp(j):
        return [pltpu.make_async_copy(dwb.at[j % 2, i], o.at[:, cols(j, FT)], s_dw.at[i, j % 2])
                for i, o in enumerate((dwg_h, dwu_h, dwd_h))]

    x_cp(0).start()
    c_cp[0].start()

    def mean8(v):
        return jnp.sum(v, axis=0, keepdims=True) * (1.0 / D)

    def colmean(rows):
        return mean8(_total(rows(r, 32) for r in range(0, D, 32)))

    def rstd(rows, mu):
        return lax.rsqrt(colmean(lambda r, n: jnp.square(rows(r, n) - mu)) + EPS)

    def group_rows(g):
        qs = _CLASSES[4 * g - 4:4 * g] if g else _CLASSES[16:]
        rows = [pl.ds(144 * (q % 2) + q // 2, 16, stride=9) for q in qs]
        return [(p, r) for p in range(2) for r in rows + ([] if g else [pl.ds(288, 16)])]

    def d_fwd(t, rows):
        parts = [_dft9([rows(64 * a + b0, 8) for a in range(9)]) for b0 in range(0, 64, 8)]
        for g in (1, 2, 3, 4):
            u = jnp.concatenate([p[i] for i in (2 * g - 1, 2 * g) for p in parts], axis=0)
            z = _nn(md[g], u.astype(bf16))
            for n, (p, r) in enumerate(group_rows(g)):
                Z[p, t, r, :] = z[16 * n:16 * n + 16]
        z = _nn(md[0, :96, :64], jnp.concatenate([p[0] for p in parts], axis=0).astype(bf16))
        for n, (p, r) in enumerate(group_rows(0)):
            Z[p, t, r, :] = z[16 * n:16 * n + 16]

    def d_inv(t):
        def spec(g):
            return jnp.concatenate([Z[p, t, r, :] for p, r in group_rows(g)], axis=0).astype(bf16)
        v = [_nn(md[5, :64, :96], spec(0))]
        for g in (1, 2, 3, 4):
            y = _nn(md[5 + g], spec(g))
            v += [y[:64], y[64:]]
        yield jnp.sum(v[0], axis=0, keepdims=True) * (1.0 / 64)
        for b0 in range(0, 64, 8):
            for a, y in enumerate(_idft9([x[b0:b0 + 8] for x in v])):
                yield 64 * a + b0, y

    def s_radix16(inverse):
        p, q = (1, 0) if inverse else (0, 1)

        def one(i):
            r = cols(i, 8)
            y = _dft16([(Z[p, a, r, :], Z[q, a, r, :]) for a in range(16)])
            for a in range(16):
                Z[p, a, r, :] = y[a][0]
                Z[q, a, r, :] = y[a][1]

        def r_body(i, _):
            for k in range(9):
                one(9 * i + k)
        lax.fori_loop(0, 4, r_body, None)
        one(36)

    def s_fwd(r):
        z = jnp.concatenate([Z[0, r], Z[1, r]], axis=1).astype(bf16)
        return _nn(z, ms[r])

    def s_inv(r, yr, yi):
        y = _nt(jnp.concatenate([yr, yi], axis=1).astype(bf16), ms[r])
        Z[0, r] = y[:, :128]
        Z[1, r] = y[:, 128:]

    c_cp[0].wait()

    def a_body(c, _):
        x_cp(c).wait()

        stages = ([x_cp(1), x_cp(2)], [x_cp(3), c_cp[1]], [c_cp[2]], [c_cp[3]])
        for n, cps in enumerate(stages):
            @pl.when(c == n)
            def _():
                for cp in cps:
                    cp.start()

        for i in range(CH // 128):
            t = c * (CH // 128) + i
            k = cols(t, 128)
            rows = lambda r, n: xT[r:r + n, k].astype(f32)
            mu = colmean(rows)
            st1[0:1, k] = mu
            st1[1:2, k] = rstd(rows, mu)

        def a1_body(i, _):
            for t in (c * 4 + n for n in range(4)):
                k = cols(t, 128)
                mu, rs = st1[0:1, k], st1[1:2, k]
                d_fwd(t, lambda r, n: (xT[r:r + n, k].astype(f32) - mu) * rs)
        pl.when(c >= 0)(lambda: a1_body(0, None))
    lax.fori_loop(0, NC, a_body, None)

    lane = lax.broadcasted_iota(jnp.int32, (8, 128), 1)

    def shift_tiles(v, sign):
        for b in (1, 2, 4, 8):
            v = [jnp.where((lane & b) != 0, v[(i + sign * b) % 16], v[i]) for i in range(16)]
        return v

    def to_spectral_order(v):
        v = shift_tiles([pltpu.roll(x, t, 1) if t else x for t, x in enumerate(v)], 1)
        return [v[-r % 16] for r in range(16)]

    def from_spectral_order(v):
        v = shift_tiles([v[-r % 16] for r in range(16)], -1)
        return [pltpu.roll(x, 128 - t, 1) if t else x for t, x in enumerate(v)]

    def lo(v):
        return pltpu.bitcast(v << 16, f32)

    def hi(v):
        return pltpu.bitcast(v & jnp.uint32(0xFFFF0000), f32)

    def w_body(i, _):
        for h in (3 * i, 3 * i + 1, 3 * i + 2):
            for p, w in enumerate((wr, wi)):
                v = [pltpu.bitcast(w[cols(h, 16), cols(t, 128)], u32) for t in range(NT)]
                for r, x in enumerate(to_spectral_order(v)):
                    Wp[r, p, cols(h, 8), :] = lo(x)
                    Wp[r, p, cols(18 + h, 8), :] = hi(x)

    s_radix16(False)
    c_cp[1].wait()
    c_cp[2].wait()
    for cp in [c_cp[4]] + g_cp:
        cp.start()
    lax.fori_loop(0, 6, w_body, None)
    first = lax.broadcasted_iota(jnp.int32, (8, 128), 0) == 0
    for p, w in enumerate((wr, wi)):
        v = [jnp.where(first, w[288:289, cols(t, 128)].astype(f32), 0.0) for t in range(NT)]
        for r, x in enumerate(to_spectral_order(v)):
            Wp[r, p, 288:296, :] = x
            Wp[r, p, 296:304, :] = jnp.zeros((8, 128), f32)

    c_cp[3].wait()

    def pair(i):
        t0 = i // (HS // 128) * (2 * HS // 128) + i % (HS // 128)
        return t0, t0 + HS // 128

    def operand_sums(i, v0, v1, c_t, c_n, full=None):
        def tr(v):
            return pltpu.bitcast(v.astype(bf16).T, u32)

        for h in range(0, HD, 16):
            a11, a21, a12, a22 = v0(h, 16), v0(HD + h, 16), v1(h, 16), v1(HD + h, 16)
            if full is not None:
                c0, c1 = [cols(t, 128) for t in pair(i)]
                full[h:h + 16, c0], full[HD + h:HD + h + 16, c0] = a11.astype(bf16), a21.astype(bf16)
                full[h:h + 16, c1], full[HD + h:HD + h + 16, c1] = a12.astype(bf16), a22.astype(bf16)
            for m, v in enumerate((a11 + a22, a21 + a22, a11 + a12, a21 - a11, a12 - a22)):
                c_t[m, h:h + 16, cols(i, 128)] = v.astype(bf16)
        for m, slots in enumerate(_PASSES):
            v = [_left(slot, lambda h, r: (v0, v1)[h](r, 64)) for slot in slots]
            c_n[cols(i, 64), 128 * m:128 * m + 128] = tr(jnp.concatenate(v, axis=0))

    def c_filter(i):
        xs = [s_fwd(4 * i + k) for k in range(4)]
        for k in range(4):
            s_inv(4 * i + k, *c_one(4 * i + k, xs[k]))

    def c_body(i, _):
        c_filter(i)
        acc_n[:, cols(i, 1024)] = jnp.zeros((D, 1024), f32)

    def cg_body(i, _):
        c_filter(2 + i)
        for h in (4 * i + k for k in range(4)):
            v0, v1 = [lambda r, n, t=t: gT[r:r + n, cols(t, 128)].astype(f32) for t in pair(h)]
            operand_sums(h, v0, v1, gTc, gc)
            for t, v in zip(pair(h), (v0, v1)):
                st2[5:6, cols(t, 128)] = colmean(lambda r, n: jnp.square(v(r, n)))

    def c_one(r, x):
        Xs[r] = x.astype(bf16)
        xr, xi, w_r, w_i = x[:, :128], x[:, 128:], Wp[r, 0], Wp[r, 1]
        return xr * w_r - xi * w_i, xr * w_i + xi * w_r
    lax.fori_loop(0, 2, c_body, None)
    for cp in [c_cp[4]] + g_cp:
        cp.wait()
    for cp in w_cp(0) + w_cp(1):
        cp.start()
    lax.fori_loop(0, 2, cg_body, None)
    s_radix16(True)

    def e_body(i, _):
        for t in (4 * i + n for n in range(4)):
            k = cols(t, 128)
            pieces = d_inv(t)
            mu = st1[0:1, k] + next(pieces)
            tot = [0.0] * 3
            for n, (r, y) in enumerate(pieces):
                h = xT[r:r + 8, k].astype(f32) + y
                acc_o[r:r + 8, k] = h
                tot[n % 3] = tot[n % 3] + jnp.square(h - mu)
            st2[0:1, k] = mu
            var = mean8(_total(tot))
            st2[1:2, k] = lax.rsqrt(var + EPS)
            st2[4:5, k] = var
    lax.fori_loop(0, NT // 4, e_body, None)

    def n_body(i, _):
        ns = [(acc_o[:, k] - st2[0:1, k]) * st2[1:2, k] for k in (cols(t, 128) for t in pair(i))]
        v0, v1 = [lambda r, n, x=x: x[r:r + n] for x in ns]
        operand_sums(i, v0, v1, n2Tc, n2c, n2T)
    lax.fori_loop(0, NT // 2, n_body, None)

    def tile_ok(j, ok=1.0):
        for w in (wg, wu, wd):
            col, row = 0.0, []
            for r in range(0, D, 16):
                sq = jnp.square(w[j, r:r + 16, :].astype(f32))
                col = col + sq
                row.append(jnp.sum(sq[:, :HF] + sq[:, HF:], axis=1, keepdims=True))
            ok = ok * _balanced(jnp.sum(col, axis=0, keepdims=True))
            ok = ok * _balanced(jnp.concatenate(row, axis=0))
        return ok.astype(jnp.int32)[0, 0]

    def f_step(j, ffn):
        @pl.when(j + 1 < NJ)
        def _():
            for cp in w_cp(j + 1):
                cp.wait()

        @pl.when(j >= 2)
        def _():
            for cp in dw_cp(j - 2):
                cp.wait()

        @pl.when(j + 2 < NJ)
        def _():
            for cp in w_cp(j + 2):
                cp.start()

        ok = ffn(j)
        for cp in dw_cp(j):
            cp.start()
        return ok

    def ffn_plain(j):
        acc_w[...] = jnp.zeros(acc_w.shape, f32)

        def body(t, _):
            k = cols(t, 128)
            n, g = n2T[:, k], gT[:, k]
            da, du, p = [x.astype(bf16) for x in _swiglu(_tn(wg[j], n), _tn(wu[j], n), _tn(wd[j], g))]
            acc_o[:, k] += _nn(wd[j], p)
            acc_n[:, k] += _nn(wg[j], da) + _nn(wu[j], du)
            for i, (lhs, rhs) in enumerate(((n, da), (n, du), (g, p))):
                acc_w[i] += _nt(lhs, rhs)
        lax.fori_loop(0, NT, body, None)
        dwb[j % 2] = acc_w[...].astype(bf16)

    def ffn_strassen(j):
        def combine(m1, m2, m3, m4, m5, m6, m7):
            return m1 + m4 - m5 + m7, m3 + m5, m2 + m4, m1 - m2 + m3 + m6

        def rhs_sums(w):
            def blk(h, r):
                return w[j, r:r + 64, h * HF:(h + 1) * HF].astype(f32)
            return [jnp.concatenate([_right(slot, blk) for slot in slots], axis=0).astype(bf16)
                    for slots in _PASSES]

        def lhs_sums(w):
            v = w[j].astype(f32)
            a11, a12, a21, a22 = v[:HD, :HF], v[:HD, HF:], v[HD:, :HF], v[HD:, HF:]
            sums = [x.astype(bf16) for x in (a11 - a22, a21 - a22, a11 - a12, a11 - a21, a12 - a22)]
            return sums[:2] + [w[j, :HD, :HF], w[j, HD:, HF:]] + sums[2:]

        def proj(u, cn, wc):
            m = {k: _nn(pltpu.bitcast(cn[cols(u, HS // 2), 128 * k:128 * k + 128], bf16), wc[k])
                 for k in _ORDER}
            return _quadrants(*[m[k] for k in range(16)])

        def sums(p, q, r, t):
            return [x.astype(bf16) for x in (p + t, p, q - t, r - p, t, p + q, r + t)]

        wr_g, wr_u, wr_d = rhs_sums(wg), rhs_sums(wu), rhs_sums(wd)
        das, dus, ps = [], [], []
        for u in range(NU):
            quads = [_swiglu(*q) for q in
                     zip(proj(u, n2c, wr_g), proj(u, n2c, wr_u), proj(u, gc, wr_d))]
            for dst, q in zip((das, dus, ps), zip(*quads)):
                dst.append(sums(*q))

        wl_g, wl_u, wl_d = lhs_sums(wg), lhs_sums(wu), lhs_sums(wd)

        def back(u, acc, terms):
            m2, m4, n3, m5, m1, m7, m6 = [
                _total(_nt(w[m], c[k]) for w, c in terms)
                for m, k in ((1, 1), (3, 5), (2, 6), (4, 4), (0, 0), (6, 2), (5, 3))]
            s0, s1 = cols(2 * u, HS), cols(2 * u + 1, HS)
            acc[:HD, s0] += m4 - m5 + m1 + m7
            acc[:HD, s1] += n3 - m5
            acc[HD:, s0] += m2 + m4
            acc[HD:, s1] += m2 + n3 - m1 - m6

        def wgrad(i, full, ct, cs):
            def lhs(u):
                sc = cols(u, HS)
                return [ct[0, :, sc], ct[1, :, sc], full[:HD, cols(2 * u, HS)],
                        full[HD:, cols(2 * u + 1, HS)], ct[2, :, sc], ct[3, :, sc], ct[4, :, sc]]
            ls = [lhs(u) for u in range(NU)]
            c11, c12, c21, c22 = combine(*[_total(_nn(ls[u][m], cs[u][m]) for u in range(NU))
                                           for m in range(7)])
            dwb[j % 2, i, :HD, :HF] = c11.astype(bf16)
            dwb[j % 2, i, :HD, HF:] = c12.astype(bf16)
            dwb[j % 2, i, HD:, :HF] = c21.astype(bf16)
            dwb[j % 2, i, HD:, HF:] = c22.astype(bf16)

        for u in range(NU):
            back(u, acc_o, [(wl_d, ps[u])])
            back(u, acc_n, [(wl_g, das[u]), (wl_u, dus[u])])
        ok = tile_ok(jnp.minimum(j + 1, NJ - 1))
        wgrad(0, n2T, n2Tc, das)
        wgrad(1, n2T, n2Tc, dus)
        wgrad(2, gT, gTc, ps)
        return ok

    for cp in w_cp(0):
        cp.wait()
    rs2 = jnp.square(st2[1:2, :])
    tokens_ok = _balanced(rs2) * _balanced(st2[4:5, :] * rs2) * _balanced(st2[5:6, :])
    done, _ = lax.while_loop(lambda c: (c[0] < NJ) & (c[1] > 0),
                             lambda c: (c[0] + 1, f_step(c[0], ffn_strassen)),
                             (jnp.int32(0), tile_ok(0, tokens_ok)))

    def plain_body(j, _):
        f_step(j, ffn_plain)
    lax.fori_loop(done, NJ, plain_body, None)

    def m_body(i, _):
        k = cols(i, 512)
        m1 = m2 = 0.0
        for r in range(0, D, 16):
            outb[r:r + 16, k] = acc_o[r:r + 16, k].astype(bf16)
            dn = acc_n[r:r + 16, k]
            m1, m2 = m1 + dn, m2 + dn * n2T[r:r + 16, k].astype(f32)
        st2[2:3, k], st2[3:4, k] = mean8(m1), mean8(m2)
    lax.fori_loop(0, S // 512, m_body, None)
    o_cp = pltpu.make_async_copy(outb, out_h, s_o.at[0])
    o_cp.start()

    def a2_body(i, _):
        for t in (4 * i + n for n in range(4)):
            k = cols(t, 128)
            rs, m1, m2 = st2[1:2, k], st2[2:3, k], st2[3:4, k]

            def rows(r, n):
                dn = acc_n[r:r + n, k] - m1 - n2T[r:r + n, k].astype(f32) * m2
                dh = gT[r:r + n, k].astype(f32) + rs * dn
                acc_n[r:r + n, k] = dh
                return dh
            d_fwd(t, rows)
    lax.fori_loop(0, NT // 4, a2_body, None)
    s_radix16(False)

    rowk = lax.broadcasted_iota(jnp.int32, (144, 128), 0)

    def c2_body(i, _):
        gs = [s_fwd(4 * i + k) for k in range(4)]
        for k in range(4):
            c2_one(4 * i + k, gs[k])

    def c2_one(r, gs):
        gr, gi, w_r, w_i = gs[:, :128], gs[:, 128:], Wp[r, 0], Wp[r, 1]
        s_inv(r, gr * w_r + gi * w_i, gi * w_r - gr * w_i)
        xr, xi = Xs[r, :, :128].astype(f32), Xs[r, :, 128:].astype(f32)
        for p, d in enumerate((xr * gr + xi * gi, xr * gi - xi * gr)):
            even = d[:144] * jnp.where(rowk == 0, 1.0 / (S * D), 2.0 / (S * D))
            T[r, p, :144] = pltpu.pack_elementwise([even, d[144:288] * (2.0 / (S * D))],
                                                   packed_dtype=bf16).astype(u32)
            T[r, p, 144:] = pltpu.bitcast(d[288:296] * (1.0 / (S * D)), u32)
    lax.fori_loop(0, 4, c2_body, None)

    def dw_body(i, _):
        for h in (3 * i, 3 * i + 1, 3 * i + 2):
            for p, w in enumerate((dwr, dwi)):
                v = from_spectral_order([T[r, p, cols(h, 8), :] for r in range(16)])
                for t in range(NT):
                    w[cols(h, 16), cols(t, 128)] = pltpu.bitcast(v[t], bf16)
    lax.fori_loop(0, 6, dw_body, None)
    for p, w in enumerate((dwr, dwi)):
        v = from_spectral_order([T[r, p, 144:, :] for r in range(16)])
        for t in range(NT):
            w[288:289, cols(t, 128)] = pltpu.bitcast(v[t], f32)[:1].astype(bf16)
    dwr_cp = pltpu.make_async_copy(dwr, dwr_h, s_o.at[1])
    dwi_cp = pltpu.make_async_copy(dwi, dwi_h, s_o.at[2])
    dwr_cp.start()
    dwi_cp.start()
    s_radix16(True)

    def dx_cp(i):
        return pltpu.make_async_copy(dxb.at[:, cols(i, 256)], dx_h.at[:, cols(i, 256)], s_o.at[3 + i])

    def e2_body(i, _):
        for t in (4 * i + n for n in range(4)):
            k = cols(t, 128)
            mu = st1[0:1, k]
            pieces = d_inv(t)
            st1[2:3, k] = next(pieces)
            t2 = [0.0] * 3
            for n, (r, y) in enumerate(pieces):
                acc_o[r:r + 8, k] = y
                t2[n % 3] = t2[n % 3] + y * (xT[r:r + 8, k].astype(f32) - mu)
            st1[3:4, k] = mean8(_total(t2))

        def dx_body(n, _):
            k = cols(2 * i + n, 256)
            mu, rs, m1 = st1[0:1, k], st1[1:2, k], st1[2:3, k]
            m2 = st1[3:4, k] * rs * rs
            for r in range(0, D, 16):
                xc = (xT[r:r + 16, k].astype(f32) - mu) * m2
                dxb[r:r + 16, k] = (acc_n[r:r + 16, k]
                                    + rs * (acc_o[r:r + 16, k] - m1 - xc)).astype(bf16)
            dx_cp(2 * i + n).start()
        lax.fori_loop(0, 2, dx_body, None)
    lax.fori_loop(0, NT // 4, e2_body, None)

    for j in (NJ - 2, NJ - 1):
        for cp in dw_cp(j):
            cp.wait()
    for cp in [o_cp, dwr_cp, dwi_cp] + [dx_cp(i) for i in range(NT // 2)]:
        cp.wait()


@jax.jit
def pallas_sequential_preLN__spectral_gfnet__swiglu_ffn__prompt_kernel(
    A_x: jax.Array,
    A_w_r: jax.Array,
    A_w_i: jax.Array,
    B_x: jax.Array,
    B_w_gate: jax.Array,
    B_w_up: jax.Array,
    B_w_down: jax.Array,
    grad_out: jax.Array,
):
    del B_x
    sds = jax.ShapeDtypeStruct
    vm = pltpu.VMEM
    hbm = pl.BlockSpec(memory_space=pl.ANY)
    dma = pltpu.SemaphoreType.DMA
    out, dx, dwr, dwi, dwg, dwu, dwd = pl.pallas_call(
        _kernel,
        in_specs=[hbm] * 9,
        out_specs=[hbm] * 7,
        out_shape=[sds((D, S), bf16)] * 2 + [sds((DF, S), bf16)] * 2 + [sds((D, F), bf16)] * 3,
        scratch_shapes=[
            vm((D, S), bf16), vm((D, S), bf16), vm((DF, S), bf16), vm((DF, S), bf16),
            vm((NJ, D, FT), bf16), vm((NJ, D, FT), bf16), vm((NJ, D, FT), bf16),
            vm((10, 128, 128), bf16), vm((16, 256, 256), bf16),
            vm((D, S), bf16), vm((D, S), bf16), vm((DF, S), bf16), vm((DF, S), bf16),
            vm((2, 3, D, FT), bf16),
            vm((D, S), bf16),
            vm((5, HD, S // 2), bf16), vm((5, HD, S // 2), bf16),
            vm((S // 4, 2048), u32), vm((S // 4, 2048), u32),
            vm((D, S), f32), vm((D, S), f32), vm((3, D, FT), f32),
            vm((2, NT, KR, 128), f32), vm((16, KR, 256), bf16), vm((16, 2, KR, 128), f32),
            vm((16, 2, 152, 128), u32), vm((8, S), f32), vm((8, S), f32),
            dma((4,)), dma((NU,)), dma((5,)), dma((3, NJ)), dma((3, 2)), dma((11,)),
        ],
        compiler_params=pltpu.CompilerParams(vmem_limit_bytes=120 * 2**20),
    )(A_x[0].T, A_w_r.T, A_w_i.T, B_w_gate, B_w_up, B_w_down.T, grad_out[0].T, _MD, _MS)
    return out.T[None], dx.T[None], dwr.T, dwi.T, dwg, dwu, dwd.T
```
